```python
import os as _os
_os.environ.setdefault("JAX_PLATFORMS", "cpu")
import jax
import jax.numpy as jnp

def _softmax(x, axis=-1):
    return jax.nn.softmax(x, axis=axis)
def _gelu(x):
    return jax.nn.gelu(x, approximate=True)
def _silu(x):
    return jax.nn.silu(x)
def _sigmoid(x):
    return jax.nn.sigmoid(x)
def _layernorm(x, axis=-1, eps=1e-5):
    m = jnp.mean(x, axis=axis, keepdims=True)
    v = jnp.var(x, axis=axis, keepdims=True)
    return (x - m) / jnp.sqrt(v + eps)
def _scatter_add(tgt, idx, src, axis=0):
    return tgt.at[idx].add(src)
def _segment_sum(src, seg, n):
    return jax.ops.segment_sum(src, seg, n)
class _Rng:
    def __init__(self, key):
        self._k = key
    def _next(self):
        self._k, sub = jax.random.split(self._k)
        return sub
    def normal(self, shape):
        return jax.random.normal(self._next(), shape, dtype=jnp.bfloat16)
    def randint(self, lo, hi, shape):
        return jax.random.randint(self._next(), shape, lo, hi, dtype=jnp.int32)
    def uniform(self, shape, lo=0.0, hi=1.0):
        return jax.random.uniform(self._next(), shape, jnp.bfloat16, lo, hi)
    def permutation(self, n):
        return jax.random.permutation(self._next(), n)


kernel_name = 'gated_mix__mha_block__mixer_s_mlp__prompt'

def setup_inputs():
    _rng = _Rng(jax.random.key(int.from_bytes(__import__("os").urandom(4), "little")))
    _w = (lambda a: (lambda t: t.astype(jnp.bfloat16) if jnp.issubdtype(t.dtype, jnp.floating) else t)(jnp.asarray(a)))
    def _A_setup():
        B, S, D, H = 1, 2048, 512, 32
        return {
            "x": _w((lambda *s: _rng.normal(s) * 0.05)(B, S, D)),
            "wqkv": _w((lambda *s: _rng.normal(s) * 0.8)(D, 3 * D)),
            "wo": _w((lambda *s: _rng.normal(s) * 0.05)(D, D)),
        }
    _A_in = _A_setup()

    def _B_setup():
        B, S, D, F = 1, 2048, 512, 1792
        return {
            "x":  _w((lambda *s: _rng.normal(s) * 0.05)(B, S, D)),
            "w1": _w((lambda *s: _rng.normal(s) * 0.2)(D, D) * (D ** -0.5)),
            "w2": _w((lambda *s: _rng.normal(s) * 0.2)(D, D) * (D ** -0.5)),
            "w3": _w((lambda *s: _rng.normal(s) * 0.2)(D, F) * (D ** -0.5)),
            "w4": _w((lambda *s: _rng.normal(s) * 0.2)(F, D) * (F ** -0.5)),
        }
    _B_in = _B_setup()

    return {
        "A_x": _A_in["x"],
        "A_wqkv": _A_in["wqkv"],
        "A_wo": _A_in["wo"],
        "B_x": _B_in["x"],
        "B_w1": _B_in["w1"],
        "B_w2": _B_in["w2"],
        "B_w3": _B_in["w3"],
        "B_w4": _B_in["w4"],
        "gate_w": _w((lambda *s: _rng.normal(s) * 0.05)(512) * 16.0),
    }

def reference(A_x, A_wqkv, A_wo, B_x, B_w1, B_w2, B_w3, B_w4, gate_w):
    def _A_ref(x, wqkv, wo):
        B, S, D = x.shape
        H = 32
        Dh = D // H
        qkv = (lambda x, *d: x.transpose(*d))((x @ wqkv).reshape(B, S, 3, H, Dh), 2, 0, 3, 1, 4)
        q, k, v = qkv[0], qkv[1], qkv[2]
        scores = jnp.einsum("bhqd,bhkd->bhqk", q, k) * (Dh ** -0.5)
        p = _softmax(scores, axis=-1)
        o = jnp.einsum("bhqk,bhkd->bhqd", p, v)
        return (lambda x, *d: x.transpose(*d))(o, 0, 2, 1, 3).reshape(B, S, D) @ wo

    def _B_ref(x, w1, w2, w3, w4):
        B, S, D = x.shape
        h = _gelu(_layernorm(x, axis=-1) @ w1)
        c = D // 4
        g0 = jnp.pad(h[:, :, 0*c:1*c], ((0, 0), (1, 0), (0, 0)))[:, :S, :]
        g1 = jnp.pad(h[:, :, 1*c:2*c], ((0, 0), (0, 1), (0, 0)))[:, 1:, :]
        g2 = jnp.pad(h[:, :, 2*c:3*c], ((0, 0), (2, 0), (0, 0)))[:, :S, :]
        g3 = jnp.pad(h[:, :, 3*c:   ], ((0, 0), (0, 2), (0, 0)))[:, 2:, :]
        hs = jnp.concatenate([g0, g1, g2, g3], axis=-1) @ w2
        x1 = x + hs
        h2 = _gelu(_layernorm(x1, axis=-1) @ w3) @ w4
        return x1 + h2

    x = A_x
    g = _sigmoid((x * gate_w).sum(-1, keepdims=True))
    a = _A_ref(x, A_wqkv, A_wo)
    b = _B_ref(x, B_w1, B_w2, B_w3, B_w4)
    return g * a + (1 - g) * b
```

```python
import functools
import math

import jax
import jax.numpy as jnp
from jax import lax
import jax.experimental.pallas as pl
import jax.experimental.pallas.tpu as pltpu

S, D, H, DH, FF = 2048, 512, 32, 16, 1792
F32, BF16 = jnp.float32, jnp.bfloat16

NH = 2
KT = 128
QB = 512
NC = QB // 128
LAG = 2
VR = 16
DEP = 2
FINE = (2, 5, 8, 11)
NOV = (1, 2)
TL = (2, 2, 2)
CR = S * NH // H
PLAN = {0: 'u0'}
TAIL = 'u1 a0.16 u2 u3 m d0 b0.16 d1 d2 d3'
RB = 512
QSCALE = (DH ** -0.5) * math.log2(math.e)
L_MIN = 2.0 ** -40
L_MAX = 2.0 ** 20

_NT = (((1,), (1,)), ((), ()))


def _dot(a, b):
    return jnp.dot(a, b, preferred_element_type=F32)


def _gelu(x):
    c = math.sqrt(2.0 / math.pi)
    return 0.5 * x * (1.0 + jnp.tanh(c * (x + 0.044715 * (x * x * x))))


def _layernorm(x, pace=None):
    m = jnp.mean(x, axis=-1, keepdims=True)
    if pace is not None:
        m = m + jnp.tile(pace[:, 0:1], (x.shape[0] // 8, 1))
    d = x - m
    v = jnp.mean(d * d, axis=-1, keepdims=True)
    return d * lax.rsqrt(v + 1e-5)


def _kernel(ax_h, wqkv_h, wo_h, w1_h, w2_h, w3_h, w4_h, gw_h, out_h,
            ax, wqkv, wo, w1, w2, w3, w4, gw, outv,
            kt, qe, qf, vt, nmx, kext, kb, xn, ot, hb, bb, x1n, h2s, kn, wt, todo, lmin, sem, osem):
    nrb = S // RB

    def cp_x(r):
        return pltpu.make_async_copy(ax_h.at[pl.ds(r * RB, RB)], ax.at[pl.ds(r * RB, RB)], sem.at[r])

    def cp_w(j):
        return pltpu.make_async_copy(wqkv_h.at[:, pl.ds(j * D, D)], wqkv.at[j], sem.at[4 + j])

    cw1, cw2, cw3, cw4, cwo, cgw = [pltpu.make_async_copy(s, d, sem.at[7 + i]) for i, (s, d) in enumerate(
        [(w1_h, w1), (w2_h, w2), (w3_h, w3), (w4_h, w4), (wo_h, wo), (gw_h, gw.at[pl.ds(0, D)])])]
    stages = [[cp_w(1), cp_x(0)], [cp_w(0), cp_x(1)], [cp_x(2), cp_x(3), cp_w(2), cw1, cw2], [cw3, cw4], [cwo, cgw]]
    for st in stages:
        for c in st:
            c.start()

    def arrive(n):
        for c in stages[n]:
            c.wait()

    onehot8 = (lax.broadcasted_iota(jnp.int32, (8, KT), 0) == 0).astype(F32)

    tok = [None] * 4

    def done(x):
        tok.append(jnp.minimum(jnp.abs(x[0:8, 0:128]), 0.0))
        return x

    def prep_k(h):
        one = jnp.concatenate([onehot8 + tok[-TL[0]], jnp.zeros_like(onehot8)], axis=0).astype(BF16)
        for t in range(S // KT):
            kx = jnp.concatenate([kt[h * DH:(h + 1) * DH, t * KT:(t + 1) * KT], one], axis=0).T
            kext[h, t * KT // 2:(t + 1) * KT // 2, :] = pltpu.bitcast(kx, jnp.int32)

    def prep_b(h, j, ds=range(DH)):
        if VR:
            lo = [(t + 1) * KT - VR for t in range(S // KT)]
            x = jnp.concatenate([kext[h, a // 2:(a + VR) // 2, :] for a in lo], axis=0)
            x = pltpu.bitcast(x, BF16).astype(F32)
            for d in ds:
                kb[j, d, 0:x.shape[0]] = jnp.broadcast_to(x[:, d:d + 1], (x.shape[0], 128))

    def rows(r):
        return slice(r * RB, (r + 1) * RB)

    G = 128
    ng = D // G

    def grp(g):
        return slice(g * G, (g + 1) * G)

    def proj_t(j, g, r):
        if r == 0:
            for c in range(ng):
                wt[j, grp(g), grp(c)] = wqkv[j, grp(c), grp(g)].T
        return done(lax.dot_general(wt[j, grp(g), :], ax[rows(r), :], _NT, preferred_element_type=F32))

    def proj_k(g, r):
        k32 = proj_t(1, g, r)
        kt[grp(g), rows(r)] = k32.astype(BF16)
        n2 = jnp.sum((k32 * k32).reshape(G // DH, DH, RB), axis=1)
        n2 = functools.reduce(jnp.maximum, [n2[:, c:c + 128] for c in range(0, RB, 128)])
        hs = slice(g * 8, g * 8 + 8)
        kn[hs] = n2 if r == 0 else jnp.maximum(kn[hs], n2)

    def proj_q(g, r):
        qe[grp(g), rows(r)] = (proj_t(0, g, r) * QSCALE).astype(BF16)

    def proj_v(g, r):
        vt[grp(g), rows(r)] = proj_t(2, g, r).astype(BF16)

    def bound(g, r):
        hs = slice(g * 8, g * 8 + 8)
        kmax2 = jnp.max(kn[hs] + tok[-TL[1]], axis=1, keepdims=True)
        q32 = qe[grp(g), rows(r)].astype(F32).reshape(G // DH, DH, RB)
        qf[hs, :, rows(r)] = q32
        nm = -(jnp.sqrt(jnp.sum(q32 * q32, axis=1) * kmax2) * (1.0 + 2.0 ** -6))
        nm = nm.astype(BF16).astype(F32)
        nmx[hs, :, rows(r)] = jnp.broadcast_to(nm[:, None, :], (8, 8, RB))

    def norm1(u):
        xn[grp(u), :] = _layernorm(ax[grp(u), :].astype(F32), tok[-TL[2]]).astype(BF16)

    def proj_h(u):
        hb[u * G + 8:(u + 1) * G + 8, :] = _gelu(done(_dot(xn[grp(u), :], w1[...])))

    def shift(u):
        for j, off in enumerate((7, 9, 6, 10)):
            win = pltpu.roll(hb[u * G:(u + 1) * G + 16, grp(j)], G + 16 - off, 0)
            xn[grp(u), grp(j)] = win[:G].astype(BF16)

    def mix(i):
        i0 = pl.multiple_of(i * CR, CR)
        x1 = ax[pl.ds(i0, CR), :].astype(F32) + _dot(xn[pl.ds(i0, CR), :], w2[...])
        bb[pl.ds(i0, CR), :] = x1
        x1n[...] = _layernorm(x1).astype(BF16)

    nu = S // G
    heads_left = iter(range(H))
    arrive(0)
    hb[0:8, :] = jnp.zeros((8, D), F32)
    hb[S + 8:S + 16, :] = jnp.zeros((8, D), F32)
    norm1(0)
    for g in range(ng):
        proj_k(g, 0)
    arrive(1)
    for g in range(ng):
        norm1(1 + g)
        proj_q(g, 0)
        proj_k(g, 1)
    for g in range(ng):
        if 1 + ng + g < 2 * ng:
            norm1(1 + ng + g)
        proj_q(g, 1)
    arrive(2)
    for n in range(2 * ng, nu):
        proj_k(n % ng, n // ng)
        norm1(n)
        proj_q(n % ng, n // ng)
    for u in range(nu):
        proj_h(u)
        prep_k(next(heads_left))
    for u in range(nu):
        shift(u)
        if u == nu - 3:
            mix(0)
        proj_v(u % ng, u // ng)
        prep_k(next(heads_left))
        bound(u // nrb, u % nrb)
        if ng <= u < ng + 8:
            for j in range(NH):
                prep_b(j, j, range(2 * (u - ng), 2 * (u - ng) + 2))
    arrive(3)

    lmin[...] = jnp.ones_like(lmin)
    row0 = lax.broadcasted_iota(jnp.int32, (8, QB), 0) == 0

    def heads(h0, fill):
        n = S // KT
        nqb = S // QB
        steps = [(j, qb, t) for j in range(NH) for qb in range(nqb) for t in range(n)]
        ps, lhist, lfin = {}, {}, {}
        o = l = qt = None
        bad = lmin[...]

        def vpu(i, g, c, pace):
            j, qb, _ = steps[i]
            h, c0 = h0 + j, qb * QB + c * 128
            acc = nmx[h, :, c0:c0 + 128]
            if i >= DEP:
                acc = jnp.minimum(acc, lhist[i - DEP][pace][:, c * 128:(c + 1) * 128])
            acc = jnp.concatenate([acc] * (VR // 8), axis=0)
            for d in range(DH):
                acc = acc + kb[j, d, g * VR:(g + 1) * VR, :] * jnp.broadcast_to(qf[h, d:d + 1, c0:c0 + 128], (VR, 128))
            return acc

        for i in range(len(steps) + LAG):
            for f in fill.get(i, ()):
                f()
            if i < len(steps):
                j, qb, t = steps[i]
                h = h0 + j
                cols = slice(qb * QB, (qb + 1) * QB)
                if t == 0:
                    r0 = pl.multiple_of(h * DH, DH)
                    mt = jnp.where(row0, nmx[h, :, cols], 0.0)
                    mt = jnp.concatenate([mt, jnp.zeros_like(mt)], axis=0).astype(BF16)
                    qt = jnp.concatenate([qe[pl.ds(r0, DH), cols], mt], axis=0)
                vr = 0 if i in NOV else VR
                s = _dot(pltpu.bitcast(kext[h, t * KT // 2:((t + 1) * KT - vr) // 2, :], BF16), qt)
                if vr:
                    s = jnp.concatenate([s, jnp.concatenate([vpu(i, t, c, FINE[c]) for c in range(NC)], axis=1)], axis=0)
                e = jnp.exp2(s)
                lh = []
                for u in range(0, KT, 8):
                    l = e[u:u + 8] if (t == 0 and u == 0) else l + e[u:u + 8]
                    lh.append(l)
                lhist[i] = lh
                if t == n - 1:
                    lfin[i] = l
                ps[i] = e.astype(BF16)
            if i >= LAG:
                j, qb, t = steps[i - LAG]
                r0 = pl.multiple_of((h0 + j) * DH, DH)
                cols = slice(qb * QB, (qb + 1) * QB)
                dd = _dot(vt[pl.ds(r0, DH), t * KT:(t + 1) * KT], ps.pop(i - LAG))
                if t == 0 and i - LAG > 0:
                    dd = dd + jnp.minimum(jnp.abs(o), 0.0)
                o = dd if t == 0 else o + dd
                if t == n - 1:
                    lt = jnp.sum(lfin[i - LAG], axis=0, keepdims=True)
                    ok = jnp.logical_and(lt >= L_MIN, lt <= L_MAX)
                    bad = jnp.where(ok, bad, 0.0)
                    ot[pl.ds(r0, DH), cols] = (o * (1.0 / lt)).astype(BF16)
        lmin[...] = bad

    groups = [(0, 512), (512, 1024), (1024, 1536), (1536, FF)]

    def body(i, carry):
        i0 = pl.multiple_of(i * CR, CR)

        def up(g):
            def f():
                lo, hi = groups[g]
                h2s[:, lo:hi] = _gelu(_dot(x1n[...], w3[:, lo:hi])).astype(BF16)
            return f

        def down(g):
            def f():
                lo, hi = groups[g]
                bb[pl.ds(i0, CR), :] += _dot(h2s[:, lo:hi], w4[lo:hi, :])
            return f

        def mixer():
            mix(jnp.minimum(i + 1, H // NH - 1))

        def prep(u):
            lo, hi = int(u[1:u.index('.')]), int(u[u.index('.') + 1:])
            j = 'ab'.index(u[0])
            return lambda: prep_b(jnp.minimum(i * NH + NH, H - NH) + j, j, range(lo, hi))

        units = dict(u0=up(0), u1=up(1), u2=up(2), u3=up(3), d0=down(0), d1=down(1), d2=down(2), d3=down(3),
                     m=mixer)
        for u in ' '.join(list(PLAN.values()) + [TAIL]).split():
            if u[0] in 'ab':
                units[u] = prep(u)
        heads(i * NH, {k: [units[u] for u in v.split()] for k, v in PLAN.items()})
        for u in TAIL.split():
            units[u]()
        return carry

    lax.fori_loop(0, H // NH, body, 0)

    arrive(4)

    def redo_attention():
        def slow_head(h, carry):
            r0 = pl.multiple_of(h * DH, DH)

            def slow_block(qb, carry2):
                c0 = pl.multiple_of(qb * 128, 128)
                q = qe[pl.ds(r0, DH), pl.ds(c0, 128)]
                q = jnp.concatenate([q, jnp.zeros_like(q)], axis=0)

                def slow_tile(t, st):
                    m0, l0, o0 = st
                    k0 = pl.multiple_of(t * 256, 256)
                    s = _dot(pltpu.bitcast(kext[h, pl.ds(pl.multiple_of(t * 128, 128), 128), :], BF16), q)
                    m1 = jnp.maximum(m0, jnp.max(s, axis=0, keepdims=True))
                    e = jnp.exp2(s - m1)
                    w = jnp.exp2(m0 - m1)
                    return (m1, w * l0 + jnp.sum(e, axis=0, keepdims=True),
                            w * o0 + _dot(vt[pl.ds(r0, DH), pl.ds(k0, 256)], e.astype(BF16)))

                init = (jnp.full((1, 128), -jnp.inf, F32), jnp.zeros((1, 128), F32), jnp.zeros((DH, 128), F32))
                _, lt, oo = lax.fori_loop(0, S // 256, slow_tile, init)
                ot[pl.ds(r0, DH), pl.ds(c0, 128)] = (oo / lt).astype(BF16)
                return carry2

            lax.fori_loop(0, S // 128, slow_block, 0)
            return carry

        lax.fori_loop(0, H, slow_head, 0)

    def cp_o(u):
        return pltpu.make_async_copy(outv.at[grp(u)], out_h.at[grp(u)], osem.at[u])

    def gate(rs):
        xn[rs, :] = ot[:, rs].T
        z = jnp.sum(ax[rs, :].astype(F32) * gw[0:D].astype(F32).reshape(1, D), axis=-1, keepdims=True)
        return 1.0 / (1.0 + jnp.exp(-z))

    def finish(p, carry):
        def emit():
            gs = [gate(grp(u)) for u in range(2)]
            for u in range(nu):
                if u + 2 < nu:
                    gs.append(gate(grp(u + 2)))
                a = _dot(xn[grp(u), :], wo[...])
                outv[grp(u), :] = (gs[u] * a + (1.0 - gs[u]) * bb[grp(u), :]).astype(BF16)
                cp_o(u).start()

        todo[0] = 1 - p

        @pl.when(p == 1)
        def _():
            @pl.when(jnp.min(lmin[...]) < 0.5)
            def _():
                redo_attention()
                for u in range(nu):
                    cp_o(u).wait()
                todo[0] = 1

        pl.when(todo[0] == 1)(emit)
        return carry

    lax.fori_loop(0, 2, finish, 0)
    for u in range(nu):
        cp_o(u).wait()


@jax.jit
def pallas_gated_mix__mha_block__mixer_s_mlp__prompt_kernel(
    A_x: jax.Array,
    A_wqkv: jax.Array,
    A_wo: jax.Array,
    B_x: jax.Array,
    B_w1: jax.Array,
    B_w2: jax.Array,
    B_w3: jax.Array,
    B_w4: jax.Array,
    gate_w: jax.Array,
):
    vm = pltpu.VMEM
    out = pl.pallas_call(
        _kernel,
        out_shape=jax.ShapeDtypeStruct((S, D), BF16),
        in_specs=[pl.BlockSpec(memory_space=pl.ANY)] * 8,
        out_specs=pl.BlockSpec(memory_space=pl.ANY),
        scratch_shapes=[
            vm((S, D), BF16), vm((3, D, D), BF16), vm((D, D), BF16),
            vm((D, D), BF16), vm((D, D), BF16), vm((D, FF), BF16), vm((FF, D), BF16),
            vm((16 * D,), BF16), vm((S, D), BF16),
            vm((D, S), BF16),
            vm((D, S), BF16),
            vm((H, DH, S), F32),
            vm((D, S), BF16),
            vm((H, 8, S), F32),
            vm((H, S // 2, 32), jnp.int32),
            vm((NH, DH, S // KT * VR + 8, 128), F32),
            vm((S, D), BF16),
            vm((D, S), BF16),
            vm((S + 16, D), F32),
            vm((S, D), F32),
            vm((CR, D), BF16),
            vm((CR, FF), BF16),
            vm((H, 128), F32),
            vm((3, D, D), BF16),
            pltpu.SMEM((1,), jnp.int32),
            vm((8, QB), F32),
            pltpu.SemaphoreType.DMA((13,)),
            pltpu.SemaphoreType.DMA((S // 128,)),
        ],
        compiler_params=pltpu.CompilerParams(vmem_limit_bytes=112 * 2 ** 20),
    )(A_x.reshape(S, D), A_wqkv, A_wo, B_w1, B_w2, B_w3, B_w4, gate_w)
    return out.reshape(1, S, D)
```
